```python
import os as _os
_os.environ.setdefault("JAX_PLATFORMS", "cpu")
import jax
import jax.numpy as jnp

def _softmax(x, axis=-1):
    return jax.nn.softmax(x, axis=axis)
def _gelu(x):
    return jax.nn.gelu(x, approximate=True)
def _silu(x):
    return jax.nn.silu(x)
def _sigmoid(x):
    return jax.nn.sigmoid(x)
def _layernorm(x, axis=-1, eps=1e-5):
    m = jnp.mean(x, axis=axis, keepdims=True)
    v = jnp.var(x, axis=axis, keepdims=True)
    return (x - m) / jnp.sqrt(v + eps)
def _scatter_add(tgt, idx, src, axis=0):
    return tgt.at[idx].add(src)
def _segment_sum(src, seg, n):
    return jax.ops.segment_sum(src, seg, n)
class _Rng:
    def __init__(self, key):
        self._k = key
    def _next(self):
        self._k, sub = jax.random.split(self._k)
        return sub
    def normal(self, shape):
        return jax.random.normal(self._next(), shape, dtype=jnp.bfloat16)
    def randint(self, lo, hi, shape):
        return jax.random.randint(self._next(), shape, lo, hi, dtype=jnp.int32)
    def uniform(self, shape, lo=0.0, hi=1.0):
        return jax.random.uniform(self._next(), shape, jnp.bfloat16, lo, hi)
    def permutation(self, n):
        return jax.random.permutation(self._next(), n)


kernel_name = 'recurrent_scan__sliding_block__dense_activation_mish__prompt'

def setup_inputs():
    _rng = _Rng(jax.random.key(int.from_bytes(__import__("os").urandom(4), "little")))
    _w = (lambda a: (lambda t: t.astype(jnp.bfloat16) if jnp.issubdtype(t.dtype, jnp.floating) else t)(jnp.asarray(a)))
    def _A_setup():
        B, S, D = 1, 2048, 576
        return {
            "x": _w((lambda *s: _rng.normal(s) * 0.05)(B, S, D)),
            "wqkv": _w((lambda *s: _rng.normal(s) * 0.1)(D, 3 * D)),
            "wo": _w((lambda *s: _rng.normal(s) * 0.1)(D, D)),
        }
    _A_in = _A_setup()

    def _B_setup():
        B, S, D, F = 1, 2048, 576, 4608
        return {
            "x": _w((lambda *s: _rng.normal(s) * 0.05)(B, S, D)),
            "w1": _w((lambda *s: _rng.normal(s) * 0.05)(D, F) * (D ** -0.5)),
            "b1": _w((lambda *s: _rng.normal(s) * 0.05)(F)),
            "w2": _w((lambda *s: _rng.normal(s) * 0.05)(F, D) * (F ** -0.5)),
        }
    _B_in = _B_setup()

    return {
        "A_x": _A_in["x"],
        "A_wqkv": _A_in["wqkv"],
        "A_wo": _A_in["wo"],
        "B_x": _B_in["x"],
        "B_w1": _B_in["w1"],
        "B_b1": _B_in["b1"],
        "B_w2": _B_in["w2"],
    }

def reference(A_x, A_wqkv, A_wo, B_x, B_w1, B_b1, B_w2):
    def _A_ref(x, wqkv, wo):
        B, S, D = x.shape
        H = 32; Dh = D // H; W = 256
        qkv = (lambda x, *d: x.transpose(*d))((x @ wqkv).reshape(B, S, 3, H, Dh), 2, 0, 3, 1, 4)
        q, k, v = qkv[0], qkv[1], qkv[2]
        scores = jnp.einsum("bhqd,bhkd->bhqk", q, k) * (Dh ** -0.5)
        idx = jnp.arange(S)
        mask = (idx[:, None] - idx[None, :] >= 0) & (idx[:, None] - idx[None, :] < W)
        scores = jnp.where(mask[None, None], scores, -1e9)
        p = _softmax(scores, axis=-1)
        o = jnp.einsum("bhqk,bhkd->bhqd", p, v)
        return (lambda x, *d: x.transpose(*d))(o, 0, 2, 1, 3).reshape(B, S, D) @ wo

    def _B_ref(x, w1, b1, w2):
        h = jnp.einsum("bsd,df->bsf", x, w1) + b1
        sp = jnp.log1p(jnp.exp(-jnp.abs(h))) + jnp.where(h > 0, h, jnp.zeros_like(h))
        act = h * jnp.tanh(sp)
        return jnp.einsum("bsf,fd->bsd", act, w2)

    x = A_x
    xn = _layernorm(x, axis=-1)
    s = _A_ref(xn, A_wqkv, A_wo)
    g = _silu(_B_ref(xn, B_w1, B_b1, B_w2))
    return x + s * g
```

```python
import functools
import math

import jax
import jax.numpy as jnp
from jax import lax
import jax.experimental.pallas as pl
import jax.experimental.pallas.tpu as pltpu

_H = 32
_W = 256
_T = 256
_FC = 512
_NT = (((1,), (1,)), ((), ()))
_F32 = jnp.float32
_BF16 = jnp.bfloat16


def _body(x_ref, b1_ref, wqkv_hbm, wo_hbm, w1_hbm, w2_hbm, o_ref,
          wqkv_v, wo_v, w1_v, w2_v, wqvT, woT, w2T, ks, vTs, xn_s, sT_s, sems,
          *, S, D, F):
    T = _T
    n = S // T
    Dh = D // _H
    i = pl.program_id(0)
    koff = D % 128
    kbase = D - koff
    nkt = (koff + D) // 128
    qscale = (Dh ** -0.5) * math.log2(math.e)

    cp_qkv = pltpu.make_async_copy(wqkv_hbm, wqkv_v, sems.at[0])
    cp_wo = pltpu.make_async_copy(wo_hbm, wo_v, sems.at[1])
    cp_w2 = pltpu.make_async_copy(w2_hbm, w2_v, sems.at[2])
    cp_w1 = pltpu.make_async_copy(w1_hbm, w1_v, sems.at[3])

    def attention(first):
        r0 = 0 if first else pl.multiple_of(i * T, T)
        x = x_ref[...].astype(_F32)
        mu = jnp.mean(x, axis=-1, keepdims=True)
        xc = x - mu
        var = jnp.mean(xc * xc, axis=-1, keepdims=True)
        xn = (xc * lax.rsqrt(var + 1e-5)).astype(_BF16)
        xn_s[pl.ds(r0, T), :] = xn
        kk = jnp.dot(xn, wqkv_v[:, kbase:kbase + nkt * 128],
                     preferred_element_type=_F32)
        lane = lax.broadcasted_iota(jnp.int32, (T, 128), 1)
        for c in range(nkt):
            ks[c, pl.ds(r0, T), :] = kk[:, c * 128:(c + 1) * 128].astype(_BF16)
        for c in range(nkt - 1):
            m = jnp.where(lane < 64, kk[:, (c + 1) * 128:(c + 2) * 128],
                          kk[:, c * 128:(c + 1) * 128])
            ks[nkt + c, pl.ds(r0, T), :] = m.astype(_BF16)
        qvT = lax.dot_general(wqvT[...], xn, _NT, preferred_element_type=_F32)
        row = lax.broadcasted_iota(jnp.int32, (32, T), 0)
        qw = []
        for h in range(_H):
            a = (Dh * h) // 16 * 16
            off = Dh * h - a
            inh = (row >= off) & (row < off + Dh)
            qw.append(jnp.where(inh, qvT[a:a + 32, :] * qscale, 0.0).astype(_BF16))
            srow = (off + Dh) % 32
            vw = jnp.where(row == srow, 1.0, qvT[D + a:D + a + 32, :])
            for t in range(T // 128):
                vTs[h, i * (T // 128) + t] = vw[:, t * 128:(t + 1) * 128].astype(_BF16)

        kr = lax.broadcasted_iota(jnp.int32, (128, 128), 0)
        qc = lax.broadcasted_iota(jnp.int32, (128, 128), 1)
        upper = kr > qc
        row8 = lax.broadcasted_iota(jnp.int32, (8, 128), 0)
        for t in range(T // 128):
            nk = min(t + 1, 3) if first else 3
            tile0 = i * (T // 128) + t - (nk - 1)
            k0 = (t + 1 - nk) * 128 if first else pl.multiple_of(tile0 * 128, 128)
            pieces = [None] * (D // 8)
            for h in range(_H):
                a = (Dh * h) // 16 * 16
                off = Dh * h - a
                p0 = koff + Dh * h
                c = p0 // 128
                if (p0 + Dh - 1) // 128 != c:
                    c = nkt + c
                wpos = (koff + a) % 128
                qh = qw[h][:, t * 128:(t + 1) * 128]
                z = lambda r: jnp.zeros((r, 128), _BF16)
                if wpos + 32 <= 128:
                    parts = [z(wpos), qh, z(96 - wpos)]
                else:
                    parts = [qh[16:], z(96), qh[:16]]
                parts = [p for p in parts if p.shape[0]]
                qm = jnp.concatenate(parts, axis=0)
                s = jnp.dot(ks[c, pl.ds(k0, nk * 128), :], qm,
                            preferred_element_type=_F32)
                last = s[(nk - 1) * 128:]
                if nk == 3:
                    sm = [jnp.where(upper, s[:128], last), s[128:256]]
                else:
                    sm = [jnp.where(upper, -1e9, last)] + ([s[:128]] if nk == 2 else [])
                mx = jnp.max(sm[0], axis=0, keepdims=True)
                for u in sm[1:]:
                    mx = jnp.maximum(mx, jnp.max(u, axis=0, keepdims=True))
                p = [jnp.exp2(u - mx) for u in sm]
                if nk == 3:
                    pt = [jnp.where(upper, p[0], 0.0), p[1], jnp.where(upper, 0.0, p[0])]
                else:
                    pt = p[1:] + [p[0]]
                pT = jnp.concatenate([u.astype(_BF16) for u in pt], axis=0)
                vt = jnp.concatenate([vTs[h, tile0 + u] for u in range(nk)], axis=1)
                o = jnp.dot(vt, pT, preferred_element_type=_F32)
                srow = (off + Dh) % 32
                o = o * (1.0 / o[srow:srow + 1, :])
                for g in range(4):
                    lo, hi = max(off, 8 * g), min(off + Dh, 8 * g + 8)
                    if lo >= hi:
                        continue
                    blk = o[8 * g:8 * g + 8]
                    gi = a // 8 + g
                    if hi - lo == 8 or pieces[gi] is None:
                        pieces[gi] = blk
                    else:
                        pieces[gi] = jnp.where(row8 >= lo - 8 * g, blk, pieces[gi])
            oT = jnp.concatenate(pieces, axis=0).astype(_BF16)
            sT_s[i * (T // 128) + t] = jnp.dot(woT[...], oT, preferred_element_type=_F32)

    @pl.when(i == 0)
    def _():
        cp_qkv.start()
        cp_wo.start()
        cp_w2.start()
        cp_w1.start()
        cp_qkv.wait()
        wp = nkt * 128
        wqvT[0:D, :] = wqkv_v[:, 0:wp].T[0:D]
        wqvT[D:2 * D, :] = wqkv_v[:, 3 * D - wp:3 * D].T[wp - D:wp]
        cp_wo.wait()
        woT[...] = wo_v[...].T
        attention(True)

    @pl.when(i == 1)
    def _():
        cp_w2.wait()

    @pl.when((i > 0) & (i < n))
    def _():
        nch = n - 2
        rows = F // nch
        c = jnp.minimum(i - 1, nch - 1)
        for u in range(rows // 128):
            f0 = pl.multiple_of(c * rows + u * 128, 128)
            w2T[c * (rows // 128) + u] = w2_v[pl.ds(f0, 128), :].T
        attention(False)

    @pl.when(i == n)
    def _():
        cp_w1.wait()

    @pl.when(i >= n)
    def _():
        j = i - n
        r0 = pl.multiple_of(j * T, T)
        xn = xn_s[pl.ds(r0, T), :]
        yT = jnp.zeros((D, T), _F32)
        for c in range(F // _FC):
            sl = slice(c * _FC, (c + 1) * _FC)
            hh = jnp.dot(xn, w1_v[:, sl], preferred_element_type=_F32)
            hh = hh + b1_ref[:, sl].astype(_F32)
            e = jnp.exp(jnp.minimum(hh, 20.0))
            m = e * (e + 2.0)
            act = (hh * m / (m + 2.0)).astype(_BF16)
            w2c = jnp.concatenate(
                [w2T[c * (_FC // 128) + u] for u in range(_FC // 128)], axis=1)
            yT = yT + lax.dot_general(w2c, act, _NT, preferred_element_type=_F32)
        sT = jnp.concatenate([sT_s[j * (T // 128) + t] for t in range(T // 128)], axis=1)
        r = sT * (yT * jax.nn.sigmoid(yT))
        o_ref[...] = (x_ref[...].astype(_F32) + r.T).astype(o_ref.dtype)


@jax.jit
def pallas_recurrent_scan__sliding_block__dense_activation_mish__prompt_kernel(
    A_x, A_wqkv, A_wo, B_x, B_w1, B_b1, B_w2,
):
    del B_x
    B, S, D = A_x.shape
    F = B_w1.shape[1]
    assert B == 1
    T = _T
    n = S // T
    nkt = (D % 128 + D) // 128
    hbm = pl.BlockSpec(memory_space=pl.ANY)
    out = pl.pallas_call(
        functools.partial(_body, S=S, D=D, F=F),
        grid=(2 * n,),
        in_specs=[
            pl.BlockSpec((None, T, D), lambda i: (0, i % n, 0)),
            pl.BlockSpec((1, F), lambda i: (0, 0)),
            hbm, hbm, hbm, hbm,
        ],
        out_specs=pl.BlockSpec((None, T, D), lambda i: (0, jnp.maximum(i - n, 0), 0)),
        out_shape=jax.ShapeDtypeStruct((B, S, D), A_x.dtype),
        scratch_shapes=[
            pltpu.VMEM((D, 3 * D), _BF16),
            pltpu.VMEM((D, D), _BF16),
            pltpu.VMEM((D, F), _BF16),
            pltpu.VMEM((F, D), _BF16),
            pltpu.VMEM((2 * D, D), _BF16),
            pltpu.VMEM((D, D), _BF16),
            pltpu.VMEM((F // 128, D, 128), _BF16),
            pltpu.VMEM((2 * nkt - 1, S, 128), _BF16),
            pltpu.VMEM((_H, S // 128, 32, 128), _BF16),
            pltpu.VMEM((S, D), _BF16),
            pltpu.VMEM((S // 128, D, 128), _F32),
            pltpu.SemaphoreType.DMA((4,)),
        ],
        compiler_params=pltpu.CompilerParams(
            dimension_semantics=("arbitrary",),
            vmem_limit_bytes=100 * 1024 * 1024,
        ),
    )(A_x, B_b1.reshape(1, F), A_wqkv, A_wo, B_w1, B_w2)
    return out
```

```python
import functools
import math

import jax
import jax.numpy as jnp
from jax import lax
import jax.experimental.pallas as pl
import jax.experimental.pallas.tpu as pltpu

_H = 32
_W = 256
_T = 256
_FC = 512
_NT = (((1,), (1,)), ((), ()))
_F32 = jnp.float32
_BF16 = jnp.bfloat16


def _body(x_ref, b1_ref, wqkv_hbm, wo_hbm, w1_hbm, w2_hbm, o_ref,
          wqkv_v, wo_v, w1_v, w2T, wqvT, woT, ks, vTs, xn_s, sT_s, sems,
          *, S, D, F):
    T = _T
    n = S // T
    Dh = D // _H
    i = pl.program_id(0)
    koff = D % 128
    kbase = D - koff
    nkt = (koff + D) // 128
    qscale = (Dh ** -0.5) * math.log2(math.e)

    cp_qkv = pltpu.make_async_copy(wqkv_hbm, wqkv_v, sems.at[0])
    cp_wo = pltpu.make_async_copy(wo_hbm, wo_v, sems.at[1])
    cp_w2 = pltpu.make_async_copy(w2_hbm, w2T, sems.at[2])
    cp_w1 = pltpu.make_async_copy(w1_hbm, w1_v, sems.at[3])

    def attention(first):
        r0 = 0 if first else pl.multiple_of(i * T, T)
        x = x_ref[...].astype(_F32)
        mu = jnp.mean(x, axis=0, keepdims=True)
        xc = x - mu
        var = jnp.mean(xc * xc, axis=0, keepdims=True)
        xnT = (xc * lax.rsqrt(var + 1e-5)).astype(_BF16)
        xn = xnT.T
        xn_s[pl.ds(r0, T), :] = xn
        kk = jnp.dot(xn, wqkv_v[:, kbase:kbase + nkt * 128],
                     preferred_element_type=_F32)
        lane = lax.broadcasted_iota(jnp.int32, (T, 128), 1)
        for c in range(nkt):
            ks[c, pl.ds(r0, T), :] = kk[:, c * 128:(c + 1) * 128].astype(_BF16)
        for c in range(nkt - 1):
            m = jnp.where(lane < 64, kk[:, (c + 1) * 128:(c + 2) * 128],
                          kk[:, c * 128:(c + 1) * 128])
            ks[nkt + c, pl.ds(r0, T), :] = m.astype(_BF16)
        qvT = jnp.dot(wqvT[...], xnT, preferred_element_type=_F32)
        row = lax.broadcasted_iota(jnp.int32, (32, T), 0)
        qw = []
        for h in range(_H):
            a = (Dh * h) // 16 * 16
            off = Dh * h - a
            inh = (row >= off) & (row < off + Dh)
            qw.append(jnp.where(inh, qvT[a:a + 32, :] * qscale, 0.0).astype(_BF16))
            srow = (off + Dh) % 32
            vw = jnp.where(row == srow, 1.0, qvT[D + a:D + a + 32, :])
            for t in range(T // 128):
                vTs[h, i * (T // 128) + t] = vw[:, t * 128:(t + 1) * 128].astype(_BF16)

        kr = lax.broadcasted_iota(jnp.int32, (128, 128), 0)
        qc = lax.broadcasted_iota(jnp.int32, (128, 128), 1)
        upper = kr > qc
        row8 = lax.broadcasted_iota(jnp.int32, (8, 128), 0)
        for t in range(T // 128):
            nk = min(t + 1, 3) if first else 3
            tile0 = i * (T // 128) + t - (nk - 1)
            k0 = (t + 1 - nk) * 128 if first else pl.multiple_of(tile0 * 128, 128)
            pieces = [None] * (D // 8)
            for h in range(_H):
                a = (Dh * h) // 16 * 16
                off = Dh * h - a
                p0 = koff + Dh * h
                c = p0 // 128
                if (p0 + Dh - 1) // 128 != c:
                    c = nkt + c
                wpos = (koff + a) % 128
                qh = qw[h][:, t * 128:(t + 1) * 128]
                z = lambda r: jnp.zeros((r, 128), _BF16)
                if wpos + 32 <= 128:
                    parts = [z(wpos), qh, z(96 - wpos)]
                else:
                    parts = [qh[16:], z(96), qh[:16]]
                parts = [p for p in parts if p.shape[0]]
                qm = jnp.concatenate(parts, axis=0)
                s = jnp.dot(ks[c, pl.ds(k0, nk * 128), :], qm,
                            preferred_element_type=_F32)
                last = s[(nk - 1) * 128:]
                if nk == 3:
                    sm = [jnp.where(upper, s[:128], last), s[128:256]]
                else:
                    sm = [jnp.where(upper, -1e9, last)] + ([s[:128]] if nk == 2 else [])
                mx = jnp.max(sm[0], axis=0, keepdims=True)
                for u in sm[1:]:
                    mx = jnp.maximum(mx, jnp.max(u, axis=0, keepdims=True))
                p = [jnp.exp2(u - mx) for u in sm]
                if nk == 3:
                    pt = [jnp.where(upper, p[0], 0.0), p[1], jnp.where(upper, 0.0, p[0])]
                else:
                    pt = p[1:] + [p[0]]
                pT = jnp.concatenate([u.astype(_BF16) for u in pt], axis=0)
                vt = jnp.concatenate([vTs[h, tile0 + u] for u in range(nk)], axis=1)
                o = jnp.dot(vt, pT, preferred_element_type=_F32)
                srow = (off + Dh) % 32
                o = o * (1.0 / o[srow:srow + 1, :])
                for g in range(4):
                    lo, hi = max(off, 8 * g), min(off + Dh, 8 * g + 8)
                    if lo >= hi:
                        continue
                    blk = o[8 * g:8 * g + 8]
                    gi = a // 8 + g
                    if hi - lo == 8 or pieces[gi] is None:
                        pieces[gi] = blk
                    else:
                        pieces[gi] = jnp.where(row8 >= lo - 8 * g, blk, pieces[gi])
            oT = jnp.concatenate(pieces, axis=0).astype(_BF16)
            sT_s[i * (T // 128) + t] = jnp.dot(woT[...], oT, preferred_element_type=_F32)

    @pl.when(i == 0)
    def _():
        cp_qkv.start()
        cp_wo.start()
        cp_w2.start()
        cp_w1.start()
        cp_qkv.wait()
        wp = nkt * 128
        wqvT[0:D, :] = wqkv_v[:, 0:wp].T[0:D]
        wqvT[D:2 * D, :] = wqkv_v[:, 3 * D - wp:3 * D].T[wp - D:wp]
        cp_wo.wait()
        woT[...] = wo_v[...].T
        attention(True)

    @pl.when((i > 0) & (i < n))
    def _():
        attention(False)

    @pl.when(i == n)
    def _():
        cp_w1.wait()
        cp_w2.wait()

    @pl.when(i >= n)
    def _():
        j = i - n
        r0 = pl.multiple_of(j * T, T)
        xn = xn_s[pl.ds(r0, T), :]
        yT = jnp.zeros((D, T), _F32)
        for c in range(F // _FC):
            sl = slice(c * _FC, (c + 1) * _FC)
            hh = jnp.dot(xn, w1_v[:, sl], preferred_element_type=_F32)
            hh = hh + b1_ref[sl].astype(_F32).reshape(1, _FC)
            e = jnp.exp(jnp.minimum(hh, 20.0))
            m = e * (e + 2.0)
            act = (hh * m / (m + 2.0)).astype(_BF16)
            yT = yT + lax.dot_general(w2T[:, sl], act, _NT, preferred_element_type=_F32)
        sT = jnp.concatenate([sT_s[j * (T // 128) + t] for t in range(T // 128)], axis=1)
        r = sT * (yT * jax.nn.sigmoid(yT))
        o_ref[...] = (x_ref[...].astype(_F32) + r).astype(o_ref.dtype)


@jax.jit
def pallas_recurrent_scan__sliding_block__dense_activation_mish__prompt_kernel(
    A_x, A_wqkv, A_wo, B_x, B_w1, B_b1, B_w2,
):
    del B_x
    B, S, D = A_x.shape
    F = B_w1.shape[1]
    assert B == 1
    T = _T
    n = S // T
    nkt = (D % 128 + D) // 128
    hbm = pl.BlockSpec(memory_space=pltpu.HBM)
    out = pl.pallas_call(
        functools.partial(_body, S=S, D=D, F=F),
        grid=(2 * n,),
        in_specs=[
            pl.BlockSpec((D, T), lambda i: (0, i % n)),
            pl.BlockSpec((F,), lambda i: (0,)),
            hbm, hbm, hbm, hbm,
        ],
        out_specs=pl.BlockSpec((D, T), lambda i: (0, jnp.maximum(i - n, 0))),
        out_shape=jax.ShapeDtypeStruct((D, S), A_x.dtype),
        scratch_shapes=[
            pltpu.VMEM((D, 3 * D), _BF16),
            pltpu.VMEM((D, D), _BF16),
            pltpu.VMEM((D, F), _BF16),
            pltpu.VMEM((D, F), _BF16),
            pltpu.VMEM((2 * D, D), _BF16),
            pltpu.VMEM((D, D), _BF16),
            pltpu.VMEM((2 * nkt - 1, S, 128), _BF16),
            pltpu.VMEM((_H, S // 128, 32, 128), _BF16),
            pltpu.VMEM((S, D), _BF16),
            pltpu.VMEM((S // 128, D, 128), _F32),
            pltpu.SemaphoreType.DMA((4,)),
        ],
        compiler_params=pltpu.CompilerParams(
            dimension_semantics=("arbitrary",),
            vmem_limit_bytes=100 * 1024 * 1024,
        ),
    )(A_x.reshape(S, D).T, B_b1, A_wqkv, A_wo, B_w1, B_w2.T)
    return out.T.reshape(B, S, D)
```

```python
import functools
import math

import jax
import jax.numpy as jnp
from jax import lax
import jax.experimental.pallas as pl
import jax.experimental.pallas.tpu as pltpu

_H = 32
_W = 256
_T = 256
_G = 1
_LAG = 6
_TAIL = 2
_RS = 2
_FC = 512
_NT = (((1,), (1,)), ((), ()))
_F32 = jnp.float32
_BF16 = jnp.bfloat16


def _pipelined(first, second, lag=1):
    out = first[:lag]
    for k in range(len(second)):
        out += first[k + lag:k + lag + 1] + [second[k]]
    return out


def _body(b1_hbm, x_hbm, wqkv_hbm, wo_hbm, w1_hbm, w2_hbm, o_hbm,
          x_v, wqkv_v, wo_v, w1_v, w2T, woT, ks, vTs, xn_s, s_s, o_v, b1_ref, sems,
          *, S, D, F):
    T = _T
    n = S // T
    nt = T // 128
    nc = F // _FC
    Dh = D // _H
    nkt = pl.cdiv(D, 128)
    qscale = (Dh ** -0.5) * math.log2(math.e)

    def cols(j):
        start = j * T
        return pl.ds(start if isinstance(j, int) else pl.multiple_of(start, T), T)

    def cp_in(j):
        return pltpu.make_async_copy(x_hbm.at[:, cols(j)], x_v.at[j], sems.at[5 + j])

    def cp_out(j):
        return pltpu.make_async_copy(o_v.at[j], o_hbm.at[:, cols(j)], sems.at[5 + j])

    cp_x = [cp_in(j) for j in range(n)]
    koff = D % 128
    kbase = D - koff
    cuts = (0, kbase, kbase + nkt * 128, 3 * D)
    cp_q, cp_k, cp_v = [
        pltpu.make_async_copy(wqkv_hbm.at[:, lo:hi], wqkv_v.at[:, lo:hi], sems.at[5 + n + u])
        for u, (lo, hi) in enumerate(zip(cuts, cuts[1:]))]
    cp_wo = pltpu.make_async_copy(wo_hbm, wo_v, sems.at[1])
    cp_w1 = pltpu.make_async_copy(w1_hbm, w1_v, sems.at[2])
    cp_w2 = pltpu.make_async_copy(w2_hbm, w2T, sems.at[3])

    cp_b1 = pltpu.make_async_copy(b1_hbm, b1_ref, sems.at[4])

    def layernorm(j):
        x = x_v[j].astype(_F32)
        mu = jnp.mean(x, axis=0, keepdims=True)
        xc = x - mu
        var = jnp.mean(xc * xc, axis=0, keepdims=True)
        xn_s[j] = (xc * lax.rsqrt(var + 1e-5)).astype(_BF16).T

    def store_keys(kk, r0, rows):
        lane = lax.broadcasted_iota(jnp.int32, (rows, 128), 1)
        for c in range(nkt):
            ks[c, pl.ds(r0, rows), :] = kk[:, c * 128:(c + 1) * 128].astype(_BF16)
        for c in range(nkt - 1):
            m = jnp.where(lane < 64, kk[:, (c + 1) * 128:(c + 2) * 128],
                          kk[:, c * 128:(c + 1) * 128])
            ks[nkt + c, pl.ds(r0, rows), :] = m.astype(_BF16)

    def attention(j, _):
        @pl.when(j + 1 < n)
        def _():
            cp_in(j + 1).wait()

        st = {}
        pieces = [[None] * (D // 8) for _ in range(nt)]
        kr = lax.broadcasted_iota(jnp.int32, (64, 128), 0)
        qc = lax.broadcasted_iota(jnp.int32, (64, 128), 1)
        upper = kr > qc % 64
        row8 = lax.broadcasted_iota(jnp.int32, (8, 128), 0)
        left8 = lax.broadcasted_iota(jnp.int32, (8, 128), 1) < 64

        def rows(p):
            a = (2 * Dh * p) // 16 * 16
            return a, 2 * Dh * p - a

        qkv = jnp.dot(xn_s[j], wqkv_v[...], preferred_element_type=_F32)
        store_keys(qkv[:, kbase:kbase + nkt * 128], pl.multiple_of(_W + j * T, T), T)
        qT = (qkv[:, 0:nkt * 128] * qscale).T
        vT = qkv[:, 2 * D:3 * D].T
        row = lax.broadcasted_iota(jnp.int32, (48, 128), 0)
        left = lax.broadcasted_iota(jnp.int32, (48, 128), 1) < 64
        for t in range(nt):
            q0 = qT[:, t * 128:(t + 1) * 128]
            q1 = pltpu.roll(q0, 64, 1)
            for p in range(_H // 2):
                a, off = rows(p)
                lo = jnp.where(left, off, off + Dh)
                keep = (row >= lo) & (row < lo + Dh)
                for half, (ql, qr) in enumerate(((q0, q1), (q1, q0))):
                    st["q", t, p, half] = jnp.where(
                        keep, jnp.where(left, ql[a:a + 48], qr[a:a + 48]), 0.0)
                vTs[p, 2 + j * nt + t] = jnp.where(
                    row == (off + 2 * Dh) % 48, 1.0,
                    vT[a:a + 48, t * 128:(t + 1) * 128]).astype(_BF16)
        layernorm(jnp.minimum(j + 1, n - 1))

        def scores(t, p, half):
            k0 = pl.multiple_of((j * nt + t) * 128 + 64 * half, 64)
            a, _ = rows(p)
            p0 = koff + 2 * Dh * p
            c = p0 // 128
            if (p0 + 2 * Dh - 1) // 128 != c:
                c = nkt + c
            wpos = (koff + a) % 128
            qh = st.pop(("q", t, p, half))
            z = lambda r: jnp.zeros((r, 128), _F32)
            if wpos + 48 <= 128:
                parts = [z(wpos), qh, z(80 - wpos)]
            else:
                parts = [qh[128 - wpos:], z(80), qh[:128 - wpos]]
            qm = jnp.concatenate([u for u in parts if u.shape[0]], axis=0).astype(_BF16)
            st["s", t, p, half] = jnp.dot(ks[c, pl.ds(k0, _W + 64), :], qm,
                                          preferred_element_type=_F32)

        def attend(t, p, half):
            s = st.pop(("s", t, p, half))
            a, off = rows(p)
            s0 = jnp.where(upper, s[:64], s[_W:])
            s1 = s[64:_W]
            mx = jnp.maximum(jnp.max(s0, axis=0, keepdims=True),
                             jnp.max(s1, axis=0, keepdims=True))
            p0 = jnp.exp2(s0 - mx)
            pt = [jnp.where(upper, p0, 0.0), jnp.exp2(s1 - mx), jnp.where(upper, 0.0, p0)]
            z = [jnp.zeros((64, 128), _F32)]
            pT = jnp.concatenate(z + pt if half else pt + z, axis=0).astype(_BF16)
            vt = jnp.concatenate([vTs[p, j * nt + t + u] for u in range(3)], axis=1)
            o = jnp.dot(vt, pT, preferred_element_type=_F32)
            srow = (off + 2 * Dh) % 48
            o = o * (1.0 / o[srow:srow + 1, :])
            if half == 0:
                st["o"] = o
                return
            oa = st.pop("o")
            for g in range(6):
                lo, hi = max(off, 8 * g), min(off + 2 * Dh, 8 * g + 8)
                if lo >= hi:
                    continue
                ga, gb = oa[8 * g:8 * g + 8], o[8 * g:8 * g + 8]
                mid = off + Dh - 8 * g
                if mid >= 8:
                    blk = jnp.where(left8, ga, pltpu.roll(gb, 64, 1))
                elif mid <= 0:
                    blk = jnp.where(left8, pltpu.roll(ga, 64, 1), gb)
                else:
                    blk = jnp.where(left8 == (row8 < mid), jnp.where(left8, ga, gb),
                                    pltpu.roll(jnp.where(left8, gb, ga), 64, 1))
                gi = a // 8 + g
                if pieces[t][gi] is not None:
                    blk = jnp.where(row8 >= lo - 8 * g, blk, pieces[t][gi])
                pieces[t][gi] = blk

        def out_proj(t):
            oT = jnp.concatenate(pieces[t], axis=0).astype(_BF16)
            for r in range(0, D, D // _RS):
                rs = slice(r, r + D // _RS)
                s_s[j * nt + t, rs] = jnp.dot(woT[rs], oT, preferred_element_type=_F32)

        def group(fn, u0):
            for u in range(u0, u0 + _G):
                fn(u // _H, u % _H // 2, u % 2)

        starts = range(0, nt * _H, _G)
        tasks = _pipelined([functools.partial(group, scores, u) for u in starts],
                           [functools.partial(group, attend, u) for u in starts], _LAG)
        for t in range(nt - 1):
            tasks.insert(len(tasks) - _TAIL, functools.partial(out_proj, t))
        for f in tasks:
            f()
        out_proj(nt - 1)

    def combine(j, y):
        sT = jnp.concatenate([s_s[j * nt + t] for t in range(nt)], axis=1)
        hy = 0.5 * y
        o_v[j] = (x_v[j].astype(_F32) + sT * (hy + hy * jnp.tanh(hy))).astype(o_v.dtype)

    def ffn(j, _):
        st = {}

        def up(c):
            sl = slice(c * _FC, (c + 1) * _FC)
            hh = jnp.dot(xn_s[j], w1_v[:, sl], preferred_element_type=_F32)
            hh = hh + b1_ref[sl].astype(_F32).reshape(1, _FC)
            e = jnp.exp(jnp.minimum(hh, 20.0))
            m = e * (e + 2.0)
            st[c] = (hh * m / (m + 2.0)).astype(_BF16)

        def down(c):
            sl = slice(c * _FC, (c + 1) * _FC)
            act = st.pop(c)
            y = lax.dot_general(w2T[:, sl], act, _NT, preferred_element_type=_F32)
            st["y"] = y if c == 0 else st["y"] + y

        tasks = _pipelined([functools.partial(up, c) for c in range(nc)],
                           [functools.partial(down, c) for c in range(nc)])
        for f in tasks:
            f()
        combine(j, st["y"])
        cp_out(j).start()

    cp_x[0].start()
    cp_k.start()
    vTs[:, 0:2] = jnp.zeros((_H // 2, 2, 48, 128), _BF16)
    cp_x[0].wait()
    for c in (cp_wo, cp_q, cp_v, cp_x[1]):
        c.start()
    layernorm(0)
    cp_k.wait()
    k0 = jnp.dot(xn_s[0, 0:16, :], wqkv_v[:, kbase:kbase + nkt * 128],
                 preferred_element_type=_F32)
    store_keys(jnp.broadcast_to(k0[0:1], (_W, nkt * 128)), 0, _W)
    cp_wo.wait()
    woT[...] = wo_v[...].T
    cp_q.wait()
    cp_v.wait()
    for c in cp_x[2:] + [cp_w1, cp_w2, cp_b1]:
        c.start()
    lax.fori_loop(0, n, attention, None)
    cp_w1.wait()
    cp_w2.wait()
    cp_b1.wait()
    lax.fori_loop(0, n, ffn, None)
    for j in range(n):
        cp_out(j).wait()


@jax.jit
def pallas_recurrent_scan__sliding_block__dense_activation_mish__prompt_kernel(
    A_x, A_wqkv, A_wo, B_x, B_w1, B_b1, B_w2,
):
    del B_x
    B, S, D = A_x.shape
    F = B_w1.shape[1]
    assert B == 1
    T = _T
    n = S // T
    nkt = pl.cdiv(D, 128)
    hbm = pl.BlockSpec(memory_space=pltpu.HBM)
    out = pl.pallas_call(
        functools.partial(_body, S=S, D=D, F=F),
        in_specs=[hbm, hbm, hbm, hbm, hbm, hbm],
        out_specs=hbm,
        out_shape=jax.ShapeDtypeStruct((D, S), A_x.dtype),
        scratch_shapes=[
            pltpu.VMEM((n, D, T), _BF16),
            pltpu.VMEM((D, 3 * D), _BF16),
            pltpu.VMEM((D, D), _BF16),
            pltpu.VMEM((D, F), _BF16),
            pltpu.VMEM((D, F), _BF16),
            pltpu.VMEM((D, D), _BF16),
            pltpu.VMEM((2 * nkt - 1, _W + S, 128), _BF16),
            pltpu.VMEM((_H // 2, (_W + S) // 128, 48, 128), _BF16),
            pltpu.VMEM((n, T, D), _BF16),
            pltpu.VMEM((S // 128, D, 128), _F32),
            pltpu.VMEM((n, D, T), A_x.dtype),
            pltpu.VMEM((F,), B_b1.dtype),
            pltpu.SemaphoreType.DMA((8 + n,)),
        ],
        compiler_params=pltpu.CompilerParams(vmem_limit_bytes=100 * 1024 * 1024),
    )(B_b1, A_x.reshape(S, D).T, A_wqkv, A_wo, B_w1, B_w2.T)
    return out.T.reshape(B, S, D)
```

```python
import functools
import math

import jax
import jax.numpy as jnp
from jax import lax
import jax.experimental.pallas as pl
import jax.experimental.pallas.tpu as pltpu

_H = 32
_W = 256
_T = 256
_G = 1
_LAG = 6
_TAIL = 2
_RS = 2
_FC = 768
_NT = (((1,), (1,)), ((), ()))
_F32 = jnp.float32
_BF16 = jnp.bfloat16


def _pipelined(first, second, lag=1):
    out = first[:lag]
    for k in range(len(second)):
        out += first[k + lag:k + lag + 1] + [second[k]]
    return out


def _strassen(m):
    m1, m2, m3, m4, m5, m6, m7 = m
    return jnp.concatenate(
        [jnp.concatenate([m1 + m4 - m5 + m7, m3 + m5], axis=1),
         jnp.concatenate([m2 + m4, m1 - m2 + m3 + m6], axis=1)], axis=0)


def _body(b1_hbm, x_hbm, wqkv_hbm, wo_hbm, w1_hbm, w2_hbm, o_hbm,
          x_v, wqkv_v, wo_v, w1_v, w2T, w1c, w2c, woT, ks, vTs, xn_s, s_s, o_v, b1_ref, sems,
          *, S, D, F):
    T = _T
    n = S // T
    nt = T // 128
    nc = F // _FC
    FH = _FC // 2
    KH = D // 256 * 128
    Dh = D // _H
    nkt = pl.cdiv(D, 128)
    qscale = (Dh ** -0.5) * math.log2(math.e)

    def cols(j):
        start = j * T
        return pl.ds(start if isinstance(j, int) else pl.multiple_of(start, T), T)

    def cp_in(j):
        return pltpu.make_async_copy(x_hbm.at[:, cols(j)], x_v.at[j], sems.at[5 + j])

    def cp_out(j):
        return pltpu.make_async_copy(o_v.at[j], o_hbm.at[:, cols(j)], sems.at[5 + j])

    cp_x = [cp_in(j) for j in range(n)]
    koff = D % 128
    kbase = D - koff
    cuts = (0, kbase, kbase + nkt * 128, 3 * D)
    cp_q, cp_k, cp_v = [
        pltpu.make_async_copy(wqkv_hbm.at[:, lo:hi], wqkv_v.at[:, lo:hi], sems.at[5 + n + u])
        for u, (lo, hi) in enumerate(zip(cuts, cuts[1:]))]
    cp_wo = pltpu.make_async_copy(wo_hbm, wo_v, sems.at[1])
    cp_w1 = pltpu.make_async_copy(w1_hbm, w1_v, sems.at[2])
    cp_w2 = pltpu.make_async_copy(w2_hbm, w2T, sems.at[3])

    cp_b1 = pltpu.make_async_copy(b1_hbm, b1_ref, sems.at[4])

    def layernorm(j):
        x = x_v[j].astype(_F32)
        mu = jnp.mean(x, axis=0, keepdims=True)
        xc = x - mu
        var = jnp.mean(xc * xc, axis=0, keepdims=True)
        xn_s[j] = (xc * lax.rsqrt(var + 1e-5)).astype(_BF16).T

    def store_keys(kk, r0, rows):
        lane = lax.broadcasted_iota(jnp.int32, (rows, 128), 1)
        for c in range(nkt):
            ks[c, pl.ds(r0, rows), :] = kk[:, c * 128:(c + 1) * 128].astype(_BF16)
        for c in range(nkt - 1):
            m = jnp.where(lane < 64, kk[:, (c + 1) * 128:(c + 2) * 128],
                          kk[:, c * 128:(c + 1) * 128])
            ks[nkt + c, pl.ds(r0, rows), :] = m.astype(_BF16)

    def attention(j, _):
        @pl.when(j + 1 < n)
        def _():
            cp_in(j + 1).wait()

        st = {}
        pieces = [[None] * (D // 8) for _ in range(nt)]
        kr = lax.broadcasted_iota(jnp.int32, (64, 128), 0)
        qc = lax.broadcasted_iota(jnp.int32, (64, 128), 1)
        upper = kr > qc % 64
        row8 = lax.broadcasted_iota(jnp.int32, (8, 128), 0)
        left8 = lax.broadcasted_iota(jnp.int32, (8, 128), 1) < 64

        def rows(p):
            a = (2 * Dh * p) // 16 * 16
            return a, 2 * Dh * p - a

        qkv = jnp.dot(xn_s[j], wqkv_v[...], preferred_element_type=_F32)
        store_keys(qkv[:, kbase:kbase + nkt * 128], pl.multiple_of(_W + j * T, T), T)
        qT = (qkv[:, 0:nkt * 128] * qscale).T
        vT = qkv[:, 2 * D:3 * D].T
        row = lax.broadcasted_iota(jnp.int32, (48, 128), 0)
        left = lax.broadcasted_iota(jnp.int32, (48, 128), 1) < 64
        for t in range(nt):
            q0 = qT[:, t * 128:(t + 1) * 128]
            q1 = pltpu.roll(q0, 64, 1)
            for p in range(_H // 2):
                a, off = rows(p)
                lo = jnp.where(left, off, off + Dh)
                keep = (row >= lo) & (row < lo + Dh)
                for half, (ql, qr) in enumerate(((q0, q1), (q1, q0))):
                    st["q", t, p, half] = jnp.where(
                        keep, jnp.where(left, ql[a:a + 48], qr[a:a + 48]), 0.0)
                vTs[p, 2 + j * nt + t] = jnp.where(
                    row == (off + 2 * Dh) % 48, 1.0,
                    vT[a:a + 48, t * 128:(t + 1) * 128]).astype(_BF16)
        layernorm(jnp.minimum(j + 1, n - 1))

        def scores(t, p, half):
            k0 = pl.multiple_of((j * nt + t) * 128 + 64 * half, 64)
            a, _ = rows(p)
            p0 = koff + 2 * Dh * p
            c = p0 // 128
            if (p0 + 2 * Dh - 1) // 128 != c:
                c = nkt + c
            wpos = (koff + a) % 128
            qh = st.pop(("q", t, p, half))
            z = lambda r: jnp.zeros((r, 128), _F32)
            if wpos + 48 <= 128:
                parts = [z(wpos), qh, z(80 - wpos)]
            else:
                parts = [qh[128 - wpos:], z(80), qh[:128 - wpos]]
            qm = jnp.concatenate([u for u in parts if u.shape[0]], axis=0).astype(_BF16)
            st["s", t, p, half] = jnp.dot(ks[c, pl.ds(k0, _W + 64), :], qm,
                                          preferred_element_type=_F32)

        def attend(t, p, half):
            s = st.pop(("s", t, p, half))
            a, off = rows(p)
            s0 = jnp.where(upper, s[:64], s[_W:])
            s1 = s[64:_W]
            mx = jnp.maximum(jnp.max(s0, axis=0, keepdims=True),
                             jnp.max(s1, axis=0, keepdims=True))
            p0 = jnp.exp2(s0 - mx)
            pt = [jnp.where(upper, p0, 0.0), jnp.exp2(s1 - mx), jnp.where(upper, 0.0, p0)]
            z = [jnp.zeros((64, 128), _F32)]
            pT = jnp.concatenate(z + pt if half else pt + z, axis=0).astype(_BF16)
            vt = jnp.concatenate([vTs[p, j * nt + t + u] for u in range(3)], axis=1)
            o = jnp.dot(vt, pT, preferred_element_type=_F32)
            srow = (off + 2 * Dh) % 48
            o = o * (1.0 / o[srow:srow + 1, :])
            if half == 0:
                st["o"] = o
                return
            oa = st.pop("o")
            for g in range(6):
                lo, hi = max(off, 8 * g), min(off + 2 * Dh, 8 * g + 8)
                if lo >= hi:
                    continue
                ga, gb = oa[8 * g:8 * g + 8], o[8 * g:8 * g + 8]
                mid = off + Dh - 8 * g
                if mid >= 8:
                    blk = jnp.where(left8, ga, pltpu.roll(gb, 64, 1))
                elif mid <= 0:
                    blk = jnp.where(left8, pltpu.roll(ga, 64, 1), gb)
                else:
                    blk = jnp.where(left8 == (row8 < mid), jnp.where(left8, ga, gb),
                                    pltpu.roll(jnp.where(left8, gb, ga), 64, 1))
                gi = a // 8 + g
                if pieces[t][gi] is not None:
                    blk = jnp.where(row8 >= lo - 8 * g, blk, pieces[t][gi])
                pieces[t][gi] = blk

        def out_proj(t):
            oT = jnp.concatenate(pieces[t], axis=0).astype(_BF16)
            for r in range(0, D, D // _RS):
                rs = slice(r, r + D // _RS)
                s_s[j * nt + t, rs] = jnp.dot(woT[rs], oT, preferred_element_type=_F32)

        def group(fn, u0):
            for u in range(u0, u0 + _G):
                fn(u // _H, u % _H // 2, u % 2)

        starts = range(0, nt * _H, _G)
        tasks = _pipelined([functools.partial(group, scores, u) for u in starts],
                           [functools.partial(group, attend, u) for u in starts], _LAG)
        for t in range(nt - 1):
            tasks.insert(len(tasks) - _TAIL, functools.partial(out_proj, t))
        for f in tasks:
            f()
        out_proj(nt - 1)

    def combine(j, y):
        sT = jnp.concatenate([s_s[j * nt + t] for t in range(nt)], axis=1)
        hy = 0.5 * y
        o_v[j] = (x_v[j].astype(_F32) + sT * (hy + hy * jnp.tanh(hy))).astype(o_v.dtype)

    def ffn(j, _):
        st = {}

        a11, a12, a21, a22 = [
            xn_s[j, r:r + T // 2, k:k + KH].astype(_F32) for r in (0, T // 2) for k in (0, KH)]
        xs = [u.astype(_BF16) for u in
              (a11 + a22, a21 + a22, a11, a22, a11 + a12, a21 - a11, a12 - a22)]

        def up(c):
            sls = [slice(f0, f0 + FH) for f0 in (c * FH, F // 2 + c * FH)]
            lo, hi = sls
            rhs = (w1c[0, :, lo], w1_v[0:KH, lo], w1c[1, :, lo], w1c[2, :, lo],
                   w1_v[KH:2 * KH, hi], w1c[3, :, lo], w1c[4, :, lo])
            hh = _strassen([jnp.dot(u, w, preferred_element_type=_F32)
                            for u, w in zip(xs, rhs)])
            w = jnp.concatenate([w1_v[2 * KH:D, sl] for sl in sls], axis=1)
            hh = hh + jnp.dot(xn_s[j, :, 2 * KH:D], w, preferred_element_type=_F32)
            hh = hh + jnp.concatenate(
                [b1_ref[sl].astype(_F32).reshape(1, FH) for sl in sls], axis=1)
            e = jnp.exp(jnp.minimum(hh, 20.0))
            m = e * (e + 2.0)
            d = m + 2.0
            r = pl.reciprocal(d, approx=True)
            act = hh * m * (r * (2.0 - d * r))
            a1, a2 = act[:, :FH], act[:, FH:]
            b11, b12, b21, b22 = a1[:T // 2], a1[T // 2:], a2[:T // 2], a2[T // 2:]
            st[c] = [u.astype(_BF16) for u in
                     (b11 + b22, b11, b12 - b22, b21 - b11, b22, b11 + b12, b21 + b22)]

        def down(c):
            sl = slice(c * FH, (c + 1) * FH)
            sl2 = slice(F // 2 + c * FH, F // 2 + (c + 1) * FH)
            lhs = (w2c[0, :, sl], w2c[1, :, sl], w2T[0:D // 2, sl], w2T[D // 2:D, sl2],
                   w2c[2, :, sl], w2c[3, :, sl], w2c[4, :, sl])
            for u, (wa, act) in enumerate(zip(lhs, st.pop(c))):
                y = lax.dot_general(wa, act, _NT, preferred_element_type=_F32)
                st["m", u] = y if c == 0 else st["m", u] + y

        tasks = _pipelined([functools.partial(up, c) for c in range(nc)],
                           [functools.partial(down, c) for c in range(nc)])
        for f in tasks:
            f()
        combine(j, _strassen([st["m", u] for u in range(7)]))
        cp_out(j).start()

    cp_x[0].start()
    cp_k.start()
    vTs[:, 0:2] = jnp.zeros((_H // 2, 2, 48, 128), _BF16)
    cp_x[0].wait()
    for c in (cp_wo, cp_q, cp_v, cp_x[1]):
        c.start()
    layernorm(0)
    cp_k.wait()
    k0 = jnp.dot(xn_s[0, 0:16, :], wqkv_v[:, kbase:kbase + nkt * 128],
                 preferred_element_type=_F32)
    store_keys(jnp.broadcast_to(k0[0:1], (_W, nkt * 128)), 0, _W)
    cp_wo.wait()
    woT[...] = wo_v[...].T
    cp_q.wait()
    cp_v.wait()
    for c in cp_x[2:] + [cp_w1, cp_w2, cp_b1]:
        c.start()
    lax.fori_loop(0, n, attention, None)
    cp_w1.wait()
    cp_w2.wait()
    cp_b1.wait()

    def weight_sums(c, _):
        lo = pl.ds(pl.multiple_of(c * 256, 128), 256)
        hi = pl.ds(pl.multiple_of(F // 2 + c * 256, 128), 256)
        for r in range(0, D // 2, 16):
            top, bot = slice(r, r + 16), slice(D // 2 + r, D // 2 + r + 16)
            a11, a12 = w2T[top, lo].astype(_F32), w2T[top, hi].astype(_F32)
            a21, a22 = w2T[bot, lo].astype(_F32), w2T[bot, hi].astype(_F32)
            for u, w in enumerate((a11 + a22, a21 + a22, a11 + a12, a21 - a11, a12 - a22)):
                w2c[u, top, lo] = w.astype(_BF16)
        for r in range(0, KH, 16):
            top, bot = slice(r, r + 16), slice(KH + r, KH + r + 16)
            b11, b12 = w1_v[top, lo].astype(_F32), w1_v[top, hi].astype(_F32)
            b21, b22 = w1_v[bot, lo].astype(_F32), w1_v[bot, hi].astype(_F32)
            for u, w in enumerate((b11 + b22, b12 - b22, b21 - b11, b11 + b12, b21 + b22)):
                w1c[u, top, lo] = w.astype(_BF16)

    lax.fori_loop(0, F // 512, weight_sums, None)
    lax.fori_loop(0, n, ffn, None)
    for j in range(n):
        cp_out(j).wait()


@jax.jit
def pallas_recurrent_scan__sliding_block__dense_activation_mish__prompt_kernel(
    A_x, A_wqkv, A_wo, B_x, B_w1, B_b1, B_w2,
):
    del B_x
    B, S, D = A_x.shape
    F = B_w1.shape[1]
    assert B == 1
    T = _T
    n = S // T
    nkt = pl.cdiv(D, 128)
    hbm = pl.BlockSpec(memory_space=pltpu.HBM)
    out = pl.pallas_call(
        functools.partial(_body, S=S, D=D, F=F),
        in_specs=[hbm, hbm, hbm, hbm, hbm, hbm],
        out_specs=hbm,
        out_shape=jax.ShapeDtypeStruct((D, S), A_x.dtype),
        scratch_shapes=[
            pltpu.VMEM((n, D, T), _BF16),
            pltpu.VMEM((D, 3 * D), _BF16),
            pltpu.VMEM((D, D), _BF16),
            pltpu.VMEM((D, F), _BF16),
            pltpu.VMEM((D, F), _BF16),
            pltpu.VMEM((5, D // 256 * 128, F // 2), _BF16),
            pltpu.VMEM((5, D // 2, F // 2), _BF16),
            pltpu.VMEM((D, D), _BF16),
            pltpu.VMEM((2 * nkt - 1, _W + S, 128), _BF16),
            pltpu.VMEM((_H // 2, (_W + S) // 128, 48, 128), _BF16),
            pltpu.VMEM((n, T, D), _BF16),
            pltpu.VMEM((S // 128, D, 128), _F32),
            pltpu.VMEM((n, D, T), A_x.dtype),
            pltpu.VMEM((F,), B_b1.dtype),
            pltpu.SemaphoreType.DMA((8 + n,)),
        ],
        compiler_params=pltpu.CompilerParams(vmem_limit_bytes=100 * 1024 * 1024),
    )(B_b1, A_x.reshape(S, D).T, A_wqkv, A_wo, B_w1, B_w2.T)
    return out.T.reshape(B, S, D)
```
